```python
import jax
import jax.numpy as jnp

def _softmax(x, axis=-1):
    return jax.nn.softmax(x, axis=axis)
def _gelu(x):
    return jax.nn.gelu(x, approximate=True)
def _silu(x):
    return jax.nn.silu(x)
def _sigmoid(x):
    return jax.nn.sigmoid(x)
def _layernorm(x, axis=-1, eps=1e-5):
    m = jnp.mean(x, axis=axis, keepdims=True)
    v = jnp.var(x, axis=axis, keepdims=True)
    return (x - m) / jnp.sqrt(v + eps)
def _scatter_add(tgt, idx, src, axis=0):
    return tgt.at[idx].add(src)
def _segment_sum(src, seg, n):
    return jax.ops.segment_sum(src, seg, n)
class _Rng:
    def __init__(self, key):
        self._k = key
    def _next(self):
        self._k, sub = jax.random.split(self._k)
        return sub
    def normal(self, shape):
        return jax.random.normal(self._next(), shape, dtype=jnp.bfloat16)
    def randint(self, lo, hi, shape):
        return jax.random.randint(self._next(), shape, lo, hi, dtype=jnp.int32)
    def uniform(self, shape, lo=0.0, hi=1.0):
        return jax.random.uniform(self._next(), shape, jnp.bfloat16, lo, hi)
    def permutation(self, n):
        return jax.random.permutation(self._next(), n)


kernel_name = 'recurrent_scan__sliding_local_dilated__geglu_ffn__prompt'

def setup_inputs():
    _rng = _Rng(jax.random.key(int.from_bytes(__import__("os").urandom(4), "little")))
    _w = (lambda a: (lambda t: t.astype(jnp.bfloat16) if jnp.issubdtype(t.dtype, jnp.floating) else t)(jnp.asarray(a)))
    def _A_setup():
        B, S, D = 1, 2048, 1024
        return {
            "x": _w((lambda *s: _rng.normal(s) * 0.05)(B, S, D)),
            "wqkv": _w((lambda *s: _rng.normal(s) * 0.05)(D, 3 * D)),
            "wo": _w((lambda *s: _rng.normal(s) * 0.05)(D, D)),
        }
    _A_in = _A_setup()

    def _B_setup():
        B, S, D, F = 1, 2048, 1024, 3584
        return {
            "x": _w((lambda *s: _rng.normal(s) * 0.05)(B, S, D)),
            "w_gate": _w((lambda *s: _rng.normal(s) * 0.05)(D, F)),
            "w_up": _w((lambda *s: _rng.normal(s) * 0.05)(D, F)),
            "w_down": _w((lambda *s: _rng.normal(s) * 0.05)(F, D)),
        }
    _B_in = _B_setup()

    return {
        "A_x": _A_in["x"],
        "A_wqkv": _A_in["wqkv"],
        "A_wo": _A_in["wo"],
        "B_x": _B_in["x"],
        "B_w_gate": _B_in["w_gate"],
        "B_w_up": _B_in["w_up"],
        "B_w_down": _B_in["w_down"],
    }

def reference(A_x, A_wqkv, A_wo, B_x, B_w_gate, B_w_up, B_w_down):
    def _A_ref(x, wqkv, wo):
        B, S, D = x.shape
        H = 32; Dh = D // H
        W, dil = 8, 2
        qkv = (lambda x, *d: x.transpose(*d))((x @ wqkv).reshape(B, S, 3, H, Dh), 2, 0, 3, 1, 4)
        q, k, v = qkv[0], qkv[1], qkv[2]
        scale = Dh ** -0.5
        pos = jnp.arange(S)
        off = jnp.arange(W) * dil
        idx = pos[:, None] - off[None, :]
        mask = idx >= 0
        idx_c = jnp.where(mask, idx, 0).reshape(-1)
        kg = k[:, :, idx_c, :].reshape(B, H, S, W, Dh)
        vg = v[:, :, idx_c, :].reshape(B, H, S, W, Dh)
        logits = jnp.einsum("bhsd,bhswd->bhsw", q, kg) * scale
        logits = jnp.where(mask[None, None, :, :], logits, -1e9)
        attn = _softmax(logits, axis=-1)
        o = jnp.einsum("bhsw,bhswd->bhsd", attn, vg)
        return (lambda x, *d: x.transpose(*d))(o, 0, 2, 1, 3).reshape(B, S, D) @ wo

    def _B_ref(x, w_gate, w_up, w_down):
        return (_gelu(x @ w_gate) * (x @ w_up)) @ w_down

    x = A_x
    xn = _layernorm(x, axis=-1)
    s = _A_ref(xn, A_wqkv, A_wo)
    g = _silu(_B_ref(xn, B_w_gate, B_w_up, B_w_down))
    return x + s * g
```

```python
import functools

import jax
import jax.numpy as jnp
from jax import lax
from jax.experimental import pallas as pl
from jax.experimental.pallas import tpu as pltpu

f32 = jnp.float32
bf16 = jnp.bfloat16
u32 = jnp.uint32

S, D, F = 2048, 1024, 3584
HS, HD, HF = S // 2, D // 2, F // 2
W, DIL, DH = 8, 2, 32
HALO = 16
NQ = 3 * D // 256
NF = F // 256
NO = D // 256
RB = 80
LNB = 128
NLN = HS // LNB


def _dot(a, b):
    return jnp.dot(a, b, preferred_element_type=f32)


def _lhs_terms(a11, a12, a21, a22):
    return (a11 + a22, a21 + a22, a11, a22, a11 + a12, a21 - a11, a12 - a22)


def _strassen(a_ref, B11, B12, B21, B22):
    b11, b12, b21, b22 = (t.astype(f32) for t in (B11, B12, B21, B22))
    m1 = _dot(a_ref[0], (b11 + b22).astype(bf16))
    m2 = _dot(a_ref[1], B11)
    m3 = _dot(a_ref[2], (b12 - b22).astype(bf16))
    m4 = _dot(a_ref[3], (b21 - b11).astype(bf16))
    c21 = m2 + m4
    m5 = _dot(a_ref[4], B22)
    c12 = m3 + m5
    m6 = _dot(a_ref[5], (b11 + b12).astype(bf16))
    c22 = m1 - m2 + m3 + m6
    m7 = _dot(a_ref[6], (b21 + b22).astype(bf16))
    c11 = m1 + m4 - m5 + m7
    return c11, c12, c21, c22


def _quads(w):
    return w[:HD, :128], w[:HD, 128:], w[HD:, :128], w[HD:, 128:]


def _gelu(x):
    c = 0.7978845608028654
    return (0.5 * x) * (1.0 + jnp.tanh(x * (c + (c * 0.044715) * (x * x))))


def _silu(x):
    h = 0.5 * x
    return h + h * jnp.tanh(h)


def _permute(x):
    xs = [pltpu.bitcast(x[:, 128 * j:128 * (j + 1)], u32) for j in range(8)]
    m = lax.broadcasted_iota(jnp.int32, xs[0].shape, 1) >> 1
    r = [xs[0]] + [pltpu.roll(xs[j], 2 * j, 1) for j in range(1, 8)]
    cur = [r[(-t) % 8] for t in range(8)]
    for b in (1, 2, 4):
        mask = (m & b) != 0
        cur = [jnp.where(mask, cur[(t - b) % 8], cur[t]) for t in range(8)]
    cur = [cur[0]] + [pltpu.roll(cur[i], 128 - 2 * i, 1) for i in range(1, 8)]
    return [pltpu.bitcast(c, bf16).astype(f32) for c in cur]


def _attention(qkv_ref, k_ref, v_ref, row0, masked):
    q = _permute(qkv_ref[pl.ds(row0 + HALO, RB), 0:D])
    for ref, c0 in ((k_ref, D), (v_ref, 2 * D)):
        t = _permute(qkv_ref[pl.ds(row0, RB + HALO), c0:c0 + D])
        for i in range(8):
            ref[i] = t[i]
    lane = lax.broadcasted_iota(jnp.int32, (RB, 128), 1)
    bit0 = (lane & 1) != 0
    bit4 = (lane & 16) != 0
    logits = []
    for w in range(W):
        rows = pl.ds(HALO - DIL * w, RB)
        l = q[0] * k_ref[0, rows, :]
        for i in range(1, 8):
            l = l + q[i] * k_ref[i, rows, :]
        l = l + jnp.where(bit0, pltpu.roll(l, 1, 1), pltpu.roll(l, 127, 1))
        l = l + jnp.where(bit4, pltpu.roll(l, 16, 1), pltpu.roll(l, 112, 1))
        l = l * (DH ** -0.5)
        if masked and w > 0:
            pos = row0 + lax.broadcasted_iota(jnp.int32, (HALO, 128), 0)
            head = jnp.where(pos >= DIL * w, l[:HALO], -1e9)
            l = jnp.concatenate([head, l[HALO:]], axis=0)
        logits.append(l)
    mx = functools.reduce(jnp.maximum, logits)
    e = [jnp.exp(l - mx) for l in logits]
    inv = 1.0 / functools.reduce(jnp.add, e)
    p = [t * inv for t in e]
    out = []
    for i in range(8):
        o = p[0] * v_ref[i, pl.ds(HALO, RB), :]
        for w in range(1, W):
            o = o + p[w] * v_ref[i, pl.ds(HALO - DIL * w, RB), :]
        out.append(o)
    return out


def _kernel(x_hbm, wqkv_hbm, wo_hbm, wg_hbm, wu_hbm, wd_hbm, out_hbm,
            x_ref, xa_ref, wqkv_ref, wg_ref, wu_ref, wo_ref, wd_ref,
            qkv_ref, k_ref, v_ref, oa_ref, ha_ref, out_ref,
            x_sem, q_sem, g_sem, u_sem, o_sem, d_sem, out_sem):
    def x_copy(h, r):
        rows = pl.ds(pl.multiple_of(h * HS + r * LNB, LNB), LNB)
        return pltpu.make_async_copy(x_hbm.at[rows], x_ref.at[rows], x_sem.at[h * NLN + r])

    def col_copy(src, dst, sem, c):
        cols = pl.ds(pl.multiple_of(c * 256, 256), 256)
        return pltpu.make_async_copy(src.at[:, cols], dst.at[c], sem.at[c])

    def wo_copy(t):
        cols = pl.ds(pl.multiple_of(t * 128, 128), 128)
        return pltpu.make_async_copy(wo_hbm.at[:, cols], wo_ref.at[t], o_sem.at[t])

    def out_copy(c):
        cols = pl.ds(pl.multiple_of(c * 256, 256), 256)
        return pltpu.make_async_copy(out_ref.at[c], out_hbm.at[:, cols], out_sem.at[c])

    for r in range(NLN):
        x_copy(0, r).start()
        x_copy(1, r).start()
    for c in range(NQ):
        col_copy(wqkv_hbm, wqkv_ref, q_sem, c).start()

    def ln_step(r, carry):
        halves = []
        for h in range(2):
            x_copy(h, r).wait()
            x = x_ref[pl.ds(pl.multiple_of(h * HS + r * LNB, LNB), LNB), :].astype(f32)
            xc = x - jnp.mean(x, axis=-1, keepdims=True)
            var = jnp.mean(xc * xc, axis=-1, keepdims=True)
            halves.append(xc * lax.rsqrt(var + 1e-5))
        top, bot = halves
        rows = pl.ds(pl.multiple_of(r * LNB, LNB), LNB)
        for i, t in enumerate(_lhs_terms(top[:, :HD], top[:, HD:], bot[:, :HD], bot[:, HD:])):
            xa_ref[i, rows, :] = t.astype(bf16)
        return carry

    lax.fori_loop(0, NLN, ln_step, 0)

    for c in range(NF):
        col_copy(wg_hbm, wg_ref, g_sem, c).start()
        col_copy(wu_hbm, wu_ref, u_sem, c).start()
    for c in range(NO):
        wo_copy(2 * c).start()
        wo_copy(2 * c + 1).start()
        col_copy(wd_hbm, wd_ref, d_sem, c).start()

    def qkv_step(c2, carry):
        for c in (2 * c2, 2 * c2 + 1):
            col_copy(wqkv_hbm, wqkv_ref, q_sem, c).wait()
        for c in (2 * c2, 2 * c2 + 1):
            c11, c12, c21, c22 = _strassen(xa_ref, *_quads(wqkv_ref[c]))
            left = pl.ds(pl.multiple_of(c * 256, 256), 128)
            right = pl.ds(pl.multiple_of(c * 256 + 128, 128), 128)
            qkv_ref[HALO:HALO + HS, left] = c11.astype(bf16)
            qkv_ref[HALO:HALO + HS, right] = c12.astype(bf16)
            qkv_ref[HALO + HS:, left] = c21.astype(bf16)
            qkv_ref[HALO + HS:, right] = c22.astype(bf16)
        return carry

    lax.fori_loop(0, NQ // 2, qkv_step, 0)
    first = qkv_ref[HALO:2 * HALO, :].astype(f32)[0:1]
    qkv_ref[0:HALO, :] = jnp.broadcast_to(first, (HALO, 3 * D)).astype(bf16)

    def ffn_step(c, carry):
        col_copy(wg_hbm, wg_ref, g_sem, c).wait()
        col_copy(wu_hbm, wu_ref, u_sem, c).wait()
        g = [_gelu(t) for t in _strassen(xa_ref, *_quads(wg_ref[c]))]

        row0 = pl.multiple_of(jnp.minimum(c * RB, HS - RB), 16)
        top = _attention(qkv_ref, k_ref.at[0], v_ref.at[0], row0, True)
        bot = _attention(qkv_ref, k_ref.at[1], v_ref.at[1], row0 + HS, False)
        for j in range(4):
            for i, t in enumerate(_lhs_terms(top[j], top[4 + j], bot[j], bot[4 + j])):
                oa_ref[i, pl.ds(row0, RB), 128 * j:128 * (j + 1)] = t.astype(bf16)

        u = _strassen(xa_ref, *_quads(wu_ref[c]))
        col = pl.ds(pl.multiple_of(c * 128, 128), 128)
        for i, t in enumerate(_lhs_terms(*(a * b for a, b in zip(g, u)))):
            ha_ref[i, :, col] = t.astype(bf16)
        return carry

    lax.fori_loop(0, NF, ffn_step, 0)

    wo_words = wo_ref.bitcast(u32)

    def wo_block(t, half):
        rows = [wo_words[t, pl.ds(8 * g + i, 8, stride=64), :]
                for i in range(4 * half, 4 * half + 4) for g in range(8)]
        return pltpu.bitcast(jnp.concatenate(rows, axis=0), bf16)

    def wd_block(c, half, side):
        return jnp.concatenate(
            [wd_ref[c, 256 * j + 128 * half:256 * j + 128 * (half + 1), 128 * side:128 * (side + 1)]
             for j in range(NF)], axis=0)

    def out_step(c, carry):
        wo_copy(2 * c).wait()
        wo_copy(2 * c + 1).wait()
        col_copy(wd_hbm, wd_ref, d_sem, c).wait()
        s = _strassen(oa_ref, wo_block(2 * c, 0), wo_block(2 * c + 1, 0),
                      wo_block(2 * c, 1), wo_block(2 * c + 1, 1))
        y = _strassen(ha_ref, wd_block(c, 0, 0), wd_block(c, 0, 1),
                      wd_block(c, 1, 0), wd_block(c, 1, 1))
        for n, (st, yt) in enumerate(zip(s, y)):
            rows = slice(HS * (n // 2), HS * (n // 2 + 1))
            cols = pl.ds(pl.multiple_of(c * 256 + 128 * (n % 2), 128), 128)
            res = x_ref[rows, cols].astype(f32) + st * _silu(yt)
            out_ref[c, rows, 128 * (n % 2):128 * (n % 2 + 1)] = res.astype(bf16)
        out_copy(c).start()
        return carry

    lax.fori_loop(0, NO, out_step, 0)
    for c in range(NO):
        out_copy(c).wait()


@jax.jit
def pallas_recurrent_scan__sliding_local_dilated__geglu_ffn__prompt_kernel(
    A_x, A_wqkv, A_wo, B_x, B_w_gate, B_w_up, B_w_down,
):
    del B_x
    dma = pltpu.SemaphoreType.DMA
    out = pl.pallas_call(
        _kernel,
        in_specs=[pl.BlockSpec(memory_space=pl.ANY)] * 6,
        out_specs=pl.BlockSpec(memory_space=pl.ANY),
        out_shape=jax.ShapeDtypeStruct((S, D), bf16),
        scratch_shapes=[
            pltpu.VMEM((S, D), bf16),
            pltpu.VMEM((7, HS, HD), bf16),
            pltpu.VMEM((NQ, D, 256), bf16),
            pltpu.VMEM((NF, D, 256), bf16),
            pltpu.VMEM((NF, D, 256), bf16),
            pltpu.VMEM((2 * NO, D, 128), bf16),
            pltpu.VMEM((NO, F, 256), bf16),
            pltpu.VMEM((HALO + S, 3 * D), bf16),
            pltpu.VMEM((2, 8, HALO + RB, 128), f32),
            pltpu.VMEM((2, 8, HALO + RB, 128), f32),
            pltpu.VMEM((7, HS, HD), bf16),
            pltpu.VMEM((7, HS, HF), bf16),
            pltpu.VMEM((NO, S, 256), bf16),
            dma((2 * NLN,)), dma((NQ,)), dma((NF,)), dma((NF,)),
            dma((2 * NO,)), dma((NO,)), dma((NO,)),
        ],
        compiler_params=pltpu.CompilerParams(vmem_limit_bytes=124 * 2**20),
    )(A_x.reshape(S, D), A_wqkv, A_wo, B_w_gate, B_w_up, B_w_down)
    return out.reshape(A_x.shape)
```

```python
import functools

import jax
import jax.numpy as jnp
from jax import lax
from jax.experimental import pallas as pl
from jax.experimental.pallas import tpu as pltpu

f32 = jnp.float32
bf16 = jnp.bfloat16
u32 = jnp.uint32

S, D, F = 2048, 1024, 3584
W, DIL, DH = 8, 2, 32
HALO = 16
XB = 256
KW = 256
CW = 512
NF = F // CW
NO = D // KW
RB = 320
GB = 32


def _dot(a, b):
    return jnp.dot(a, b, preferred_element_type=f32)


def _gelu(x):
    c = 0.7978845608028654
    return (0.5 * x) * (1.0 + jnp.tanh(x * (c + (c * 0.044715) * (x * x))))


def _row_mean(tiles):
    return jnp.sum(functools.reduce(jnp.add, tiles), axis=-1, keepdims=True) * (1.0 / D)


def _permute(groups):
    groups = [[pltpu.bitcast(x, u32) for x in xs] for xs in groups]
    pair = lax.broadcasted_iota(jnp.int32, groups[0][0].shape, 1) >> 1
    groups = [[xs[0]] + [pltpu.roll(xs[j], 2 * j, 1) for j in range(1, 8)] for xs in groups]
    out = []
    for xs in groups:
        cur = [xs[-t % 8] for t in range(8)]
        for b in (1, 2, 4):
            mask = (pair & b) != 0
            cur = [jnp.where(mask, cur[(t - b) % 8], cur[t]) for t in range(8)]
        out.append([cur[0]] + [pltpu.roll(cur[i], 128 - 2 * i, 1) for i in range(1, 8)])
    return [[pltpu.bitcast(x, bf16) for x in xs] for xs in out]


def _kernel(x_hbm, wqkv_hbm, wo_hbm, wg_hbm, wu_hbm, wd_hbm, out_hbm,
            x_ref, xn_ref, wqkv_ref, wg_ref, wu_ref, wo_ref, wd_ref,
            qkv_ref, k_ref, v_ref, o_ref, h_ref,
            x_sem, q_sem, g_sem, u_sem, o_sem, d_sem, out_sem):
    def x_copy(r):
        rows = pl.ds(r * XB, XB)
        return pltpu.make_async_copy(x_hbm.at[rows], x_ref.at[rows], x_sem.at[r])

    def col_copy(src, dst, sem, c):
        width = dst.shape[-1]
        cols = pl.ds(pl.multiple_of(c * width, width), width)
        return pltpu.make_async_copy(src.at[:, cols], dst.at[c], sem.at[c])

    qkv_copy = functools.partial(col_copy, wqkv_hbm, wqkv_ref, q_sem)
    wg_copy = functools.partial(col_copy, wg_hbm, wg_ref, g_sem)
    wu_copy = functools.partial(col_copy, wu_hbm, wu_ref, u_sem)
    wo_copy = functools.partial(col_copy, wo_hbm, wo_ref, o_sem)
    wd_copy = functools.partial(col_copy, wd_hbm, wd_ref, d_sem)

    def normalize(lo, hi):
        for row in range(lo, hi, 32):
            rows = pl.ds(row, 32)
            x = [x_ref[rows, pl.ds(128 * j, 128)].astype(f32) for j in range(8)]
            mean = _row_mean(x)
            x = [t - mean for t in x]
            inv = lax.rsqrt(_row_mean([t * t for t in x]) + 1e-5)
            for j in range(8):
                xn_ref[j, rows, :] = (x[j] * inv).astype(bf16)

    def xn(lo=0, hi=S):
        return jnp.concatenate([xn_ref[j, lo:hi, :] for j in range(8)], axis=1)

    def project(c, lo=0, hi=S):
        for t in range(2):
            v = _dot(xn(lo, hi), wqkv_ref[c, :, pl.ds(128 * t, 128)])
            qkv_ref[2 * c + t, pl.ds(HALO + lo, hi - lo), :] = v.astype(bf16)

    def stage(start=(), wait=()):
        for copy in start:
            copy.start()
        for copy in wait:
            copy.wait()

    stage([x_copy(0), x_copy(1), qkv_copy(0)], [x_copy(0)])
    normalize(0, 256)
    stage([qkv_copy(1)], [x_copy(1)])
    normalize(256, 512)
    stage([qkv_copy(2), qkv_copy(3)], [qkv_copy(0)])
    project(0, 0, 512)
    stage([x_copy(2), x_copy(3)], [qkv_copy(1)])
    project(1, 0, 512)
    stage([x_copy(r) for r in range(4, 8)], [qkv_copy(2), qkv_copy(3)])
    project(2, 0, 512)
    stage((), [x_copy(2), x_copy(3)])
    normalize(512, 1024)
    project(3, 0, 512)
    project(0, 512, 1024)
    stage([qkv_copy(c) for c in range(4, 8)], [x_copy(r) for r in range(4, 8)])
    normalize(1024, 2048)
    for c in range(1, 4):
        project(c, 512, 1024)
    for c in range(4):
        project(c, 1024, 2048)

    def kv_step(i):
        @pl.when(i == 0)
        def _():
            stage([qkv_copy(c) for c in range(8, 12)])

        @pl.when(i == 1)
        def _():
            stage([wg_copy(0), wu_copy(0)])

        stage((), [qkv_copy(4 + 4 * i + c) for c in range(4)])
        base = qkv_ref.at[pl.ds(8 + 8 * i, 8)]
        weights = wqkv_ref.at[pl.ds(4 + 4 * i, 4)]
        for t in range(8):
            v = _dot(xn(), weights[t // 2, :, pl.ds(128 * (t % 2), 128)])
            base[t, pl.ds(HALO, S), :] = v.astype(bf16)
            base[t, pl.ds(0, HALO), :] = jnp.broadcast_to(v[0:1], (HALO, 128)).astype(bf16)

    pl.loop(0, 2)(kv_step)

    def ffn_step(c):
        @pl.when(c + 1 < NF)
        def _():
            stage([wg_copy(c + 1), wu_copy(c + 1)])

        @pl.when(c < NO)
        def _():
            stage([wo_copy(c), wd_copy(c)])

        stage((), [wg_copy(c), wu_copy(c)])

        row0 = pl.multiple_of(jnp.minimum(c * RB, S - RB), 16)
        qkv_rows = qkv_ref.at[:, pl.ds(row0, HALO + RB), :]
        o_rows = o_ref.at[:, pl.ds(row0, RB), :]

        def gather(start, size, which):
            groups = [[qkv_rows[8 * m + j, pl.ds(start, size), :] for j in range(8)] for m in which]
            tiles = [[t.astype(f32) for t in ts] for ts in _permute(groups)]
            for ref, ts in zip((k_ref, v_ref), tiles[-2:]):
                for i in range(8):
                    ref[i, pl.ds(start, size), :] = ts[i]
            return tiles[0]

        def attend(row):
            q = gather(HALO + row, GB, (0, 1, 2))
            windows = [pl.ds(HALO + row - DIL * w, GB) for w in range(W)]
            logits = [functools.reduce(jnp.add, [q[i] * k_ref[i, rows, :] for i in range(8)])
                      for rows in windows]
            lane = lax.broadcasted_iota(jnp.int32, (GB, 128), 1)
            for bit in (1, 16):
                mask = (lane & bit) != 0
                logits = [l + jnp.where(mask, pltpu.roll(l, bit, 1), pltpu.roll(l, 128 - bit, 1))
                          for l in logits]
            logits = [l * DH ** -0.5 for l in logits]
            if row == 0:
                pos = row0 + lax.broadcasted_iota(jnp.int32, (GB, 128), 0)
                logits = [jnp.where(pos >= DIL * w, l, -1e9) for w, l in enumerate(logits)]
            top = functools.reduce(jnp.maximum, logits)
            e = [jnp.exp(l - top) for l in logits]
            inv = 1.0 / functools.reduce(jnp.add, e)
            p = [t * inv for t in e]
            o = [functools.reduce(jnp.add, [p[w] * v_ref[i, windows[w], :] for w in range(W)]).astype(bf16)
                 for i in range(8)]
            for j, t in enumerate(_permute([o])[0]):
                o_rows[j, pl.ds(row, GB), :] = t

        gather(0, HALO, (1, 2))
        rows = list(range(0, RB, GB))
        for t in range(4):
            cols = pl.ds(128 * t, 128)
            g = _gelu(_dot(xn(), wg_ref[c, :, cols]))
            for row in rows[3 * t:3 * t + 2]:
                attend(row)
            h_ref[c, t] = (g * _dot(xn(), wu_ref[c, :, cols])).astype(bf16)
            for row in rows[3 * t + 2:3 * t + 3]:
                attend(row)

    pl.loop(0, NF)(ffn_step)

    def out_step(c):
        stage((), [wo_copy(c), wd_copy(c)])
        for t in range(2):
            cols = pl.ds(128 * t, 128)
            y = _dot(jnp.concatenate([h_ref[j // 4, j % 4] for j in range(F // 128)], axis=1), wd_ref[c, :, cols])
            g = y * jax.nn.sigmoid(y)
            s = _dot(jnp.concatenate([o_ref[j] for j in range(8)], axis=1), wo_ref[c, :, cols])
            cols = pl.ds(pl.multiple_of(KW * c + 128 * t, 128), 128)
            x_ref[:, cols] = (x_ref[:, cols].astype(f32) + s * g).astype(bf16)
            pltpu.make_async_copy(x_ref.at[:, cols], out_hbm.at[:, cols], out_sem.at[0]).start()

    pl.loop(0, NO)(out_step)
    pltpu.make_async_copy(x_ref, out_hbm, out_sem.at[0]).wait()


@jax.jit
def pallas_recurrent_scan__sliding_local_dilated__geglu_ffn__prompt_kernel(
    A_x, A_wqkv, A_wo, B_x, B_w_gate, B_w_up, B_w_down,
):
    del B_x
    dma = pltpu.SemaphoreType.DMA
    out = pl.pallas_call(
        _kernel,
        in_specs=[pl.BlockSpec(memory_space=pl.ANY)] * 6,
        out_specs=pl.BlockSpec(memory_space=pl.ANY),
        out_shape=jax.ShapeDtypeStruct((S, D), bf16),
        scratch_shapes=[
            pltpu.VMEM((S, D), bf16),
            pltpu.VMEM((8, S, 128), bf16),
            pltpu.VMEM((3 * D // KW, D, KW), bf16),
            pltpu.VMEM((NF, D, CW), bf16),
            pltpu.VMEM((NF, D, CW), bf16),
            pltpu.VMEM((NO, D, KW), bf16),
            pltpu.VMEM((NO, F, KW), bf16),
            pltpu.VMEM((24, HALO + S, 128), bf16),
            pltpu.VMEM((8, HALO + RB, 128), f32),
            pltpu.VMEM((8, HALO + RB, 128), f32),
            pltpu.VMEM((8, S, 128), bf16),
            pltpu.VMEM((NF, 4, S, 128), bf16),
            dma((S // XB,)), dma((3 * D // KW,)), dma((NF,)), dma((NF,)),
            dma((NO,)), dma((NO,)), dma((1,)),
        ],
        compiler_params=pltpu.CompilerParams(vmem_limit_bytes=120 * 2**20),
    )(A_x.reshape(S, D), A_wqkv, A_wo, B_w_gate, B_w_up, B_w_down)
    return out.reshape(A_x.shape)
```

```python
import functools

import jax
import jax.numpy as jnp
from jax import lax
from jax.experimental import pallas as pl
from jax.experimental.pallas import tpu as pltpu

f32 = jnp.float32
bf16 = jnp.bfloat16
u32 = jnp.uint32

S, D, F = 2048, 1024, 3584
W, DIL, DH = 8, 2, 32
HALO = 16
XCUT = (0, 192, 384, 640, 1280, S)
PIECE = 128
LB = 32
HEAD = 4
QT = 5
NQ = (3 * D // 128 - HEAD) // QT
KW = 256
CW = 512
NF = F // CW
NO = D // KW
RB = 304
GB = 16


def _dot(a, b):
    return jnp.dot(a, b, preferred_element_type=f32)


def _gelu(x):
    c = 0.7978845608028654
    return (0.5 * x) * (1.0 + jnp.tanh(x * (c + (c * 0.044715) * (x * x))))


def _row_mean(tiles):
    return jnp.sum(functools.reduce(jnp.add, tiles), axis=-1, keepdims=True) * (1.0 / D)


def _permute(groups):
    groups = [[pltpu.bitcast(x, u32) for x in xs] for xs in groups]
    pair = lax.broadcasted_iota(jnp.int32, groups[0][0].shape, 1) >> 1
    groups = [[xs[0]] + [pltpu.roll(xs[j], 2 * j, 1) for j in range(1, 8)] for xs in groups]
    out = []
    for xs in groups:
        cur = [xs[-t % 8] for t in range(8)]
        for b in (1, 2, 4):
            mask = (pair & b) != 0
            cur = [jnp.where(mask, cur[(t - b) % 8], cur[t]) for t in range(8)]
        out.append([cur[0]] + [pltpu.roll(cur[i], 128 - 2 * i, 1) for i in range(1, 8)])
    return [[pltpu.bitcast(x, bf16) for x in xs] for xs in out]


def _kernel(x_hbm, wqkv_hbm, wo_hbm, wg_hbm, wu_hbm, wd_hbm, out_hbm,
            x_ref, xn_ref, wqkv_ref, wg_ref, wu_ref, wo_ref, wd_ref,
            qkv_ref, k_ref, v_ref, o_ref, h_ref,
            x_sem, q_sem, w_sem):
    def x_copy(r):
        rows = pl.ds(XCUT[r], XCUT[r + 1] - XCUT[r])
        return pltpu.make_async_copy(x_hbm.at[rows], x_ref.at[rows], x_sem.at[r])

    def head_copy(t):
        return pltpu.make_async_copy(wqkv_hbm.at[:, pl.ds(128 * t, 128)], wqkv_ref.at[NQ, :, pl.ds(128 * t, 128)],
                                     q_sem.at[NQ + t])

    def qkv_copy(c):
        cols = pl.ds(pl.multiple_of(128 * (HEAD + QT * c), 128), 128 * QT)
        return pltpu.make_async_copy(wqkv_hbm.at[:, cols], wqkv_ref.at[c], q_sem.at[c])

    def col_copies(src, dst):
        width = dst.shape[-1]
        return [pltpu.make_async_copy(src.at[:, pl.ds(c * width, width)], dst.at[c], w_sem.at[0])
                for c in range(dst.shape[0])]

    later = [copy for pair in ((wg_hbm, wg_ref), (wu_hbm, wu_ref), (wo_hbm, wo_ref), (wd_hbm, wd_ref))
             for copy in col_copies(*pair)]

    def normalize(lo, hi):
        for row in range(lo, hi, LB):
            rows = pl.ds(row, LB)
            x = [x_ref[rows, pl.ds(128 * j, 128)].astype(f32) for j in range(8)]
            mean = _row_mean(x)
            x = [t - mean for t in x]
            inv = lax.rsqrt(_row_mean([t * t for t in x]) + 1e-5)
            for j in range(8):
                xn_ref[j, rows, :] = (x[j] * inv).astype(bf16)

    def xn(lo=0, hi=S):
        return jnp.concatenate([xn_ref[j, lo:hi, :] for j in range(8)], axis=1)

    def project(tiles, lo, hi):
        for t in tiles:
            v = _dot(xn(lo, hi), wqkv_ref[NQ, :, pl.ds(128 * t, 128)])
            qkv_ref[t, pl.ds(HALO + lo, hi - lo), :] = v.astype(bf16)

    def stage(start=(), wait=()):
        for copy in start:
            copy.start()
        for copy in wait:
            copy.wait()

    stage([x_copy(0), x_copy(1)], [x_copy(0)])
    normalize(0, XCUT[1])
    stage(map(head_copy, range(HEAD)), [x_copy(1)])
    normalize(XCUT[1], XCUT[2])
    stage([x_copy(2), x_copy(3)], [head_copy(0)])
    project((0,), 0, XCUT[2])
    stage([x_copy(4)], [head_copy(1), head_copy(2)])
    project((1, 2), 0, XCUT[2])
    stage([qkv_copy(0)], [head_copy(3)])
    lo = 0
    for r, copies in ((2, ()), (3, map(qkv_copy, range(1, NQ))), (4, later)):
        stage(copies, [x_copy(r)])
        cuts = [*range(XCUT[r], XCUT[r + 1] - PIECE + 1, PIECE), XCUT[r + 1]]
        normalize(cuts[0], cuts[1])
        project((3,), lo, XCUT[r])
        lo = XCUT[r]
        for i in range(len(cuts) - 1):
            if i + 2 < len(cuts):
                normalize(cuts[i + 1], cuts[i + 2])
            project((0, 1, 2), cuts[i], cuts[i + 1])
    project((3,), lo, S)

    def qkv_step(c):
        qkv_copy(c).wait()
        tiles = qkv_ref.at[pl.ds(HEAD + QT * c, QT)]
        for t in range(QT):
            v = _dot(xn(), wqkv_ref[c, :, pl.ds(128 * t, 128)])
            tiles[t, pl.ds(HALO, S), :] = v.astype(bf16)
            tiles[t, pl.ds(0, HALO), :] = jnp.broadcast_to(v[0:1], (HALO, 128)).astype(bf16)

    pl.loop(0, NQ)(qkv_step)

    stage((), later)

    def ffn_step(c):
        row0 = pl.multiple_of(jnp.minimum(c * RB, S - RB), 16)
        qkv_rows = qkv_ref.at[:, pl.ds(row0, HALO + RB), :]
        o_rows = o_ref.at[:, pl.ds(row0, RB), :]

        def gather(start, size, which):
            groups = [[qkv_rows[8 * m + j, pl.ds(start, size), :] for j in range(8)] for m in which]
            tiles = [[t.astype(f32) for t in ts] for ts in _permute(groups)]
            for ref, ts in zip((k_ref, v_ref), tiles[-2:]):
                for i in range(8):
                    ref[i, pl.ds(start, size), :] = ts[i]
            return tiles[0]

        def attend(row):
            q = gather(HALO + row, GB, (0, 1, 2))
            windows = [pl.ds(HALO + row - DIL * w, GB) for w in range(W)]
            logits = [functools.reduce(jnp.add, [q[i] * k_ref[i, rows, :] for i in range(8)])
                      for rows in windows]
            lane = lax.broadcasted_iota(jnp.int32, (GB, 128), 1)
            for bit in (1, 16):
                mask = (lane & bit) != 0
                logits = [l + jnp.where(mask, pltpu.roll(l, bit, 1), pltpu.roll(l, 128 - bit, 1))
                          for l in logits]
            logits = [l * DH ** -0.5 for l in logits]
            if row == 0:
                pos = row0 + lax.broadcasted_iota(jnp.int32, (GB, 128), 0)
                logits = [jnp.where(pos >= DIL * w, l, -1e9) for w, l in enumerate(logits)]
            top = functools.reduce(jnp.maximum, logits)
            e = [jnp.exp(l - top) for l in logits]
            inv = 1.0 / functools.reduce(jnp.add, e)
            p = [t * inv for t in e]
            o = [functools.reduce(jnp.add, [p[w] * v_ref[i, windows[w], :] for w in range(W)]).astype(bf16)
                 for i in range(8)]
            for j, t in enumerate(_permute([o])[0]):
                o_rows[j, pl.ds(row, GB), :] = t

        gather(0, HALO, (1, 2))
        rows = list(range(0, RB, GB))
        for t in range(4):
            cols = pl.ds(128 * t, 128)
            g = _gelu(_dot(xn(), wg_ref[c, :, cols]))
            for row in rows[len(rows) * 2 * t // 7:len(rows) * (2 * t + 1) // 7]:
                attend(row)
            h_ref[c, t] = (g * _dot(xn(), wu_ref[c, :, cols])).astype(bf16)
            for row in rows[len(rows) * (2 * t + 1) // 7:len(rows) * (2 * t + 2) // 7]:
                attend(row)

    pl.loop(0, NF)(ffn_step)

    def out_step(c):
        for t in range(2):
            cols = pl.ds(128 * t, 128)
            y = _dot(jnp.concatenate([h_ref[j // 4, j % 4] for j in range(F // 128)], axis=1), wd_ref[c, :, cols])
            g = y * jax.nn.sigmoid(y)
            cuts = (0, S) if t == 0 else (0, S // 2, 3 * S // 4, 7 * S // 8, S)
            for lo, hi in zip(cuts, cuts[1:]):
                s = _dot(jnp.concatenate([o_ref[j, lo:hi, :] for j in range(8)], axis=1), wo_ref[c, :, cols])
                block = (pl.ds(lo, hi - lo), pl.ds(pl.multiple_of(KW * c + 128 * t, 128), 128))
                x_ref[block] = (x_ref[block].astype(f32) + s * g[lo:hi]).astype(bf16)
                pltpu.make_async_copy(x_ref.at[block], out_hbm.at[block], w_sem.at[0]).start()

    pl.loop(0, NO)(out_step)
    pltpu.make_async_copy(x_ref, out_hbm, w_sem.at[0]).wait()


@jax.jit
def pallas_recurrent_scan__sliding_local_dilated__geglu_ffn__prompt_kernel(
    A_x, A_wqkv, A_wo, B_x, B_w_gate, B_w_up, B_w_down,
):
    del B_x
    dma = pltpu.SemaphoreType.DMA
    flags = {"XLA_TPU_EVENLY_DISTRIBUTE_CRITICAL_NODES": True}
    out = pl.pallas_call(
        _kernel,
        in_specs=[pl.BlockSpec(memory_space=pl.ANY)] * 6,
        out_specs=pl.BlockSpec(memory_space=pl.ANY),
        out_shape=jax.ShapeDtypeStruct((S, D), bf16),
        scratch_shapes=[
            pltpu.VMEM((S, D), bf16),
            pltpu.VMEM((8, S, 128), bf16),
            pltpu.VMEM((NQ + 1, D, 128 * QT), bf16),
            pltpu.VMEM((NF, D, CW), bf16),
            pltpu.VMEM((NF, D, CW), bf16),
            pltpu.VMEM((NO, D, KW), bf16),
            pltpu.VMEM((NO, F, KW), bf16),
            pltpu.VMEM((24, HALO + S, 128), bf16),
            pltpu.VMEM((8, HALO + RB, 128), f32),
            pltpu.VMEM((8, HALO + RB, 128), f32),
            pltpu.VMEM((8, S, 128), bf16),
            pltpu.VMEM((NF, 4, S, 128), bf16),
            dma((len(XCUT) - 1,)), dma((NQ + HEAD,)), dma((1,)),
        ],
        compiler_params=pltpu.CompilerParams(vmem_limit_bytes=120 * 2**20, flags=flags),
    )(A_x.reshape(S, D), A_wqkv, A_wo, B_w_gate, B_w_up, B_w_down)
    return out.reshape(A_x.shape)
```

```python
import functools

import jax
import jax.numpy as jnp
from jax import lax
from jax.experimental import pallas as pl
from jax.experimental.pallas import tpu as pltpu

f32 = jnp.float32
bf16 = jnp.bfloat16
u32 = jnp.uint32

S, D, F = 2048, 1024, 3584
W, DIL, DH = 8, 2, 32
HALO = 16

XCUT = (0, 192, 384, 640, 1280, S)
PIECE = 128
LB = 32
HEAD = 4
QT = 5
NQ = (3 * D // 128 - HEAD) // QT
CW = 512
NF = F // CW
RB = 304
GB = 16
KW = 256
NO = D // KW


def _dot(a, b):
    return jnp.dot(a, b, preferred_element_type=f32)


def _gelu(x):
    c = 0.7978845608028654
    return (0.5 * x) * (1.0 + jnp.tanh(x * (c + (c * 0.044715) * (x * x))))


def _row_mean(tiles):
    return jnp.sum(functools.reduce(jnp.add, tiles), axis=-1, keepdims=True) * (1.0 / D)


def _regroup(groups):
    groups = [[pltpu.bitcast(x, u32) for x in xs] for xs in groups]
    pair = lax.broadcasted_iota(jnp.int32, groups[0][0].shape, 1) >> 1
    groups = [[xs[0]] + [pltpu.roll(xs[j], 2 * j, 1) for j in range(1, 8)] for xs in groups]
    out = []
    for xs in groups:
        cur = [xs[-t % 8] for t in range(8)]
        for b in (1, 2, 4):
            mask = (pair & b) != 0
            cur = [jnp.where(mask, cur[(t - b) % 8], cur[t]) for t in range(8)]
        out.append([cur[0]] + [pltpu.roll(cur[i], 128 - 2 * i, 1) for i in range(1, 8)])
    return [[pltpu.bitcast(x, bf16) for x in xs] for xs in out]


def _stage(start=(), wait=()):
    for copy in start:
        copy.start()
    for copy in wait:
        copy.wait()


def _kernel(x_hbm, wqkv_hbm, wo_hbm, wg_hbm, wu_hbm, wd_hbm, out_hbm,
            x_ref, xn_ref, wqkv_ref, wg_ref, wu_ref, wo_ref, wd_ref,
            qkv_ref, k_ref, v_ref, o_ref, h_ref,
            x_sem, q_sem, w_sem):
    def x_copy(r):
        rows = pl.ds(XCUT[r], XCUT[r + 1] - XCUT[r])
        return pltpu.make_async_copy(x_hbm.at[rows], x_ref.at[rows], x_sem.at[r])

    def head_copy(t):
        cols = pl.ds(128 * t, 128)
        return pltpu.make_async_copy(wqkv_hbm.at[:, cols], wqkv_ref.at[NQ, :, cols], q_sem.at[NQ + t])

    def qkv_copy(c):
        cols = pl.ds(pl.multiple_of(128 * (HEAD + QT * c), 128), 128 * QT)
        return pltpu.make_async_copy(wqkv_hbm.at[:, cols], wqkv_ref.at[c], q_sem.at[c])

    later_copies = [
        pltpu.make_async_copy(src.at[:, pl.ds(c * dst.shape[2], dst.shape[2])], dst.at[c], w_sem.at[0])
        for src, dst in ((wg_hbm, wg_ref), (wu_hbm, wu_ref), (wo_hbm, wo_ref), (wd_hbm, wd_ref))
        for c in range(dst.shape[0])]

    def normalize(lo, hi):
        for row in range(lo, hi, LB):
            x = [x_ref[pl.ds(row, LB), pl.ds(128 * j, 128)].astype(f32) for j in range(8)]
            mean = _row_mean(x)
            x = [t - mean for t in x]
            inv = lax.rsqrt(_row_mean([t * t for t in x]) + 1e-5)
            xn_ref[pl.ds(row // 2, LB // 2), :] = pltpu.bitcast(
                jnp.concatenate([t * inv for t in x], axis=1).astype(bf16), u32)

    def xn(lo=0, hi=S):
        return pltpu.bitcast(xn_ref[lo // 2:hi // 2, :], bf16)

    def project(tiles, lo, hi):
        for t in tiles:
            v = _dot(xn(lo, hi), wqkv_ref[NQ, :, pl.ds(128 * t, 128)])
            qkv_ref[t, pl.ds(HALO + lo, hi - lo), :] = v.astype(bf16)

    _stage([x_copy(0), x_copy(1)], [x_copy(0)])
    normalize(0, XCUT[1])
    _stage(map(head_copy, range(HEAD)), [x_copy(1)])
    normalize(XCUT[1], XCUT[2])
    _stage([x_copy(2), x_copy(3)], [head_copy(0)])
    project((0,), 0, XCUT[2])
    _stage([x_copy(4)], [head_copy(1), head_copy(2)])
    project((1, 2), 0, XCUT[2])
    _stage([qkv_copy(0)], [head_copy(3)])
    lo = 0
    for r, copies in ((2, ()), (3, map(qkv_copy, range(1, NQ))), (4, ())):
        _stage(copies, [x_copy(r)])
        cuts = range(XCUT[r], XCUT[r + 1] + 1, PIECE)
        normalize(cuts[0], cuts[1])
        project((3,), lo, XCUT[r])
        lo = XCUT[r]
        for i in range(len(cuts) - 1):
            if i + 2 < len(cuts):
                normalize(cuts[i + 1], cuts[i + 2])
            project((0, 1, 2), cuts[i], cuts[i + 1])
    project((3,), lo, S)

    @pl.loop(0, NQ)
    def _(c):
        qkv_copy(c).wait()
        tiles = qkv_ref.at[pl.ds(HEAD + QT * c, QT)]
        for t in range(QT):
            v = _dot(xn(), wqkv_ref[c, :, pl.ds(128 * t, 128)])
            tiles[t, pl.ds(HALO, S), :] = v.astype(bf16)
            tiles[t, pl.ds(0, HALO), :] = jnp.broadcast_to(v[0:1], (HALO, 128)).astype(bf16)

        @pl.when(c == 0)
        def _():
            _stage(later_copies)

    _stage((), later_copies)

    @pl.loop(0, NF)
    def _(c):
        row0 = pl.multiple_of(jnp.minimum(c * RB, S - RB), 16)
        qkv_rows = qkv_ref.at[:, pl.ds(row0, HALO + RB), :]
        o_rows = o_ref.at[:, pl.ds(row0, RB), :]

        def fetch(start, size, which):
            groups = [[qkv_rows[8 * m + j, pl.ds(start, size), :] for j in range(8)] for m in which]
            tiles = [[t.astype(f32) for t in ts] for ts in _regroup(groups)]
            for ref, ts in zip((k_ref, v_ref), tiles[-2:]):
                for i in range(8):
                    ref[i, pl.ds(start, size), :] = ts[i]
            return tiles[0]

        def attend(row):
            q = fetch(HALO + row, GB, (0, 1, 2))
            windows = [pl.ds(HALO + row - DIL * w, GB) for w in range(W)]
            logits = [functools.reduce(jnp.add, [q[i] * k_ref[i, rows, :] for i in range(8)])
                      for rows in windows]
            lane = lax.broadcasted_iota(jnp.int32, (GB, 128), 1)
            for bit in (1, 16):
                mask = (lane & bit) != 0
                logits = [l + jnp.where(mask, pltpu.roll(l, bit, 1), pltpu.roll(l, 128 - bit, 1))
                          for l in logits]
            logits = [l * DH ** -0.5 for l in logits]
            if row < HALO:
                pos = row0 + row + lax.broadcasted_iota(jnp.int32, (GB, 128), 0)
                logits = [jnp.where(pos >= DIL * w, l, -1e9) for w, l in enumerate(logits)]
            top = functools.reduce(jnp.maximum, logits)
            e = [jnp.exp(l - top) for l in logits]
            inv = 1.0 / functools.reduce(jnp.add, e)
            p = [t * inv for t in e]
            o = [functools.reduce(jnp.add, [p[w] * v_ref[i, windows[w], :] for w in range(W)]).astype(bf16)
                 for i in range(8)]
            for j, t in enumerate(_regroup([o])[0]):
                o_rows[j, pl.ds(row, GB), :] = t

        def attend_part(n):
            rows = range(0, RB, GB)
            for row in rows[len(rows) * n // 7:len(rows) * (n + 1) // 7]:
                attend(row)

        fetch(0, HALO, (1, 2))
        for t in range(CW // 128):
            cols = pl.ds(128 * t, 128)
            g = _gelu(_dot(xn(), wg_ref[c, :, cols]))
            attend_part(2 * t)
            h_ref[c, t] = (g * _dot(xn(), wu_ref[c, :, cols])).astype(bf16)
            attend_part(2 * t + 1)

    @pl.loop(0, NO)
    def _(c):
        for t in range(KW // 128):
            cols = pl.ds(128 * t, 128)
            h = jnp.concatenate([h_ref[i, j] for i in range(NF) for j in range(CW // 128)], axis=1)
            y = _dot(h, wd_ref[c, :, cols])
            g = y * jax.nn.sigmoid(y)
            cuts = (0, S) if t == 0 else (0, S // 2, 3 * S // 4, 15 * S // 16, S)
            for lo, hi in zip(cuts, cuts[1:]):
                o = jnp.concatenate([o_ref[j, lo:hi, :] for j in range(8)], axis=1)
                s = _dot(o, wo_ref[c, :, cols])
                block = (pl.ds(lo, hi - lo), pl.ds(pl.multiple_of(KW * c + 128 * t, 128), 128))
                x_ref[block] = (x_ref[block].astype(f32) + s * g[lo:hi]).astype(bf16)
                pltpu.make_async_copy(x_ref.at[block], out_hbm.at[block], w_sem.at[0]).start()

    pltpu.make_async_copy(x_ref, out_hbm, w_sem.at[0]).wait()


@jax.jit
def pallas_recurrent_scan__sliding_local_dilated__geglu_ffn__prompt_kernel(
    A_x: jax.Array,
    A_wqkv: jax.Array,
    A_wo: jax.Array,
    B_x: jax.Array,
    B_w_gate: jax.Array,
    B_w_up: jax.Array,
    B_w_down: jax.Array,
):
    del B_x
    dma = pltpu.SemaphoreType.DMA
    out = pl.pallas_call(
        _kernel,
        in_specs=[pl.BlockSpec(memory_space=pl.ANY)] * 6,
        out_specs=pl.BlockSpec(memory_space=pl.ANY),
        out_shape=jax.ShapeDtypeStruct((S, D), bf16),
        scratch_shapes=[
            pltpu.VMEM((S, D), bf16),
            pltpu.VMEM((S // 2, D), u32),
            pltpu.VMEM((NQ + 1, D, 128 * QT), bf16),
            pltpu.VMEM((NF, D, CW), bf16),
            pltpu.VMEM((NF, D, CW), bf16),
            pltpu.VMEM((NO, D, KW), bf16),
            pltpu.VMEM((NO, F, KW), bf16),
            pltpu.VMEM((24, HALO + S, 128), bf16),
            pltpu.VMEM((8, HALO + RB, 128), f32),
            pltpu.VMEM((8, HALO + RB, 128), f32),
            pltpu.VMEM((8, S, 128), bf16),
            pltpu.VMEM((NF, CW // 128, S, 128), bf16),
            dma((len(XCUT) - 1,)), dma((NQ + HEAD,)), dma((1,)),
        ],
        compiler_params=pltpu.CompilerParams(
            vmem_limit_bytes=100 * 2**20,
            flags={"XLA_TPU_EVENLY_DISTRIBUTE_CRITICAL_NODES": True},
        ),
    )(A_x.reshape(S, D), A_wqkv, A_wo, B_w_gate, B_w_up, B_w_down)
    return out.reshape(A_x.shape)
```
